```python
import os as _os
_os.environ.setdefault('JAX_PLATFORMS', 'cpu')
import jax
import jax.numpy as jnp

def _softmax(x, axis=-1):
    return jax.nn.softmax(x, axis=axis)

def _gelu(x):
    return jax.nn.gelu(x, approximate=True)

def _silu(x):
    return jax.nn.silu(x)

def _sigmoid(x):
    return jax.nn.sigmoid(x)

def _layernorm(x, axis=-1, eps=1e-05):
    m = jnp.mean(x, axis=axis, keepdims=True)
    v = jnp.var(x, axis=axis, keepdims=True)
    return (x - m) / jnp.sqrt(v + eps)

def _scatter_add(tgt, idx, src, axis=0):
    return tgt.at[idx].add(src)

def _segment_sum(src, seg, n):
    return jax.ops.segment_sum(src, seg, n)

class _Rng:

    def __init__(self, key):
        self._k = key

    def _next(self):
        self._k, sub = jax.random.split(self._k)
        return sub

    def normal(self, shape):
        return jax.random.normal(self._next(), shape, dtype=jnp.bfloat16)

    def randint(self, lo, hi, shape):
        return jax.random.randint(self._next(), shape, lo, hi, dtype=jnp.int32)

    def uniform(self, shape, lo=0.0, hi=1.0):
        return jax.random.uniform(self._next(), shape, jnp.bfloat16, lo, hi)

    def permutation(self, n):
        return jax.random.permutation(self._next(), n)
kernel_name = 'adaLN_cond__linear_kernel_hedgehog__geglu_ffn__prompt'

def setup_inputs():
    _rng = _Rng(jax.random.key(int.from_bytes(__import__("os").urandom(4), "little")))
    _w = lambda a: (lambda t: t.astype(jnp.bfloat16) if jnp.issubdtype(t.dtype, jnp.floating) else t)(jnp.asarray(a))

    def _A_setup():
        B, S, D, H = (1, 2048, 512, 32)
        Dh = D // H
        return {'x': _w((lambda *s: _rng.normal(s) * 0.05)(B, S, D)), 'wqkv': _w((lambda *s: _rng.normal(s) * 0.4)(D, 3 * D)), 'w_phi': _w((lambda *s: _rng.normal(s) * 0.4)(H, Dh, Dh) * Dh ** (-0.5)), 'wo': _w((lambda *s: _rng.normal(s) * 0.05)(D, D))}
    _A_in = _A_setup()

    def _B_setup():
        B, S, D, F = (1, 2048, 512, 1792)
        return {'x': _w((lambda *s: _rng.normal(s) * 0.05)(B, S, D)), 'w_gate': _w((lambda *s: _rng.normal(s) * 0.05)(D, F)), 'w_up': _w((lambda *s: _rng.normal(s) * 0.05)(D, F)), 'w_down': _w((lambda *s: _rng.normal(s) * 0.05)(F, D))}
    _B_in = _B_setup()
    return {'A_x': _A_in['x'], 'A_wqkv': _A_in['wqkv'], 'A_w_phi': _A_in['w_phi'], 'A_wo': _A_in['wo'], 'B_x': _B_in['x'], 'B_w_gate': _B_in['w_gate'], 'B_w_up': _B_in['w_up'], 'B_w_down': _B_in['w_down'], 'c': _w((lambda *s: _rng.normal(s) * 0.05)(1, 512) * 8.0), 'w_mod': _w((lambda *s: _rng.normal(s) * 0.05)(512, 6 * 512) * 512 ** (-0.5) * 8.0)}

def reference(A_x, A_wqkv, A_w_phi, A_wo, B_x, B_w_gate, B_w_up, B_w_down, c, w_mod):

    def _A_ref(x, wqkv, w_phi, wo):
        B, S, D = x.shape
        H = 32
        Dh = D // H
        qkv = (lambda x, *d: x.transpose(*d))((x @ wqkv).reshape(B, S, 3, H, Dh), 2, 0, 3, 1, 4)
        q, k, v = (qkv[0], qkv[1], qkv[2])
        pq = jnp.einsum('bhsd,hdf->bhsf', q, w_phi)
        pk = jnp.einsum('bhsd,hdf->bhsf', k, w_phi)
        phi_q = jnp.concatenate([_softmax(pq, axis=-1), _softmax(-pq, axis=-1)], axis=-1)
        phi_k = jnp.concatenate([_softmax(pk, axis=-1), _softmax(-pk, axis=-1)], axis=-1)
        kv = jnp.einsum('bhsf,bhsd->bhfd', phi_k, v)
        z = jnp.einsum('bhsf->bhf', phi_k)
        num = jnp.einsum('bhqf,bhfd->bhqd', phi_q, kv)
        den = jnp.einsum('bhqf,bhf->bhq', phi_q, z)[..., None] + 1e-06
        o = num / den
        return (lambda x, *d: x.transpose(*d))(o, 0, 2, 1, 3).reshape(B, S, D) @ wo

    def _B_ref(x, w_gate, w_up, w_down):
        return _gelu(x @ w_gate) * (x @ w_up) @ w_down
    x = A_x
    mod = (_silu(c) @ w_mod).reshape(c.shape[0], 6, 1, -1)
    sa, ca, ga, sb, cb, gb = (mod[:, 0].copy(), mod[:, 1].copy(), mod[:, 2].copy(), mod[:, 3].copy(), mod[:, 4].copy(), mod[:, 5].copy())
    h = _layernorm(x, axis=-1) * (1 + ca) + sa
    x = x + ga * _A_ref(h, A_wqkv, A_w_phi, A_wo)
    h = _layernorm(x, axis=-1) * (1 + cb) + sb
    x = x + gb * _B_ref(h, B_w_gate, B_w_up, B_w_down)
    return x
```

```python
import jax
import jax.numpy as jnp
import jax.experimental.pallas as pl
import jax.experimental.pallas.tpu as pltpu

S, D, H, DH, F = 2048, 512, 32, 16, 1792
G = 4
T1 = 1024
T2 = 512
FC = 256
BF, F32 = jnp.bfloat16, jnp.float32
NT = (((1,), (1,)), ((), ()))
TN = (((0,), (0,)), ((), ()))


def _dot(a, b, dims=(((1,), (0,)), ((), ()))):
    return jax.lax.dot_general(a, b, dims, preferred_element_type=F32)


def _ln_mod(x, scale, shift):
    m = jnp.mean(x, axis=-1, keepdims=True)
    xc = x - m
    v = jnp.mean(xc * xc, axis=-1, keepdims=True)
    return xc * jax.lax.rsqrt(v + 1e-5) * (1.0 + scale) + shift


def _phi(p):
    t = p.shape[-1]
    p = p.reshape(DH, 8, t)
    a = jnp.exp(p - jnp.max(p, axis=0, keepdims=True))
    b = jnp.exp(jnp.min(p, axis=0, keepdims=True) - p)
    a = a * (1.0 / jnp.sum(a, axis=0, keepdims=True))
    b = b * (1.0 / jnp.sum(b, axis=0, keepdims=True))
    return jnp.concatenate(
        [a.reshape(128, t).astype(BF), b.reshape(128, t).astype(BF)], axis=0)


def _kernel(x_hbm, wqkv_hbm, wphi_ref, wo_hbm, wg_hbm, wu_hbm, wd_hbm, c_ref, wm_hbm,
            o_hbm,
            x_v, wqkv_v, wo_v, wg_v, wu_v, wd_v, wm_v, wt_v, wop_v, h_v, kv_v, out_v,
            sem, osem):
    cp = lambda s, d, i: pltpu.make_async_copy(s, d, sem.at[i])
    c_wm0 = cp(wm_hbm.at[:, pl.ds(0, 2 * D)], wm_v.at[:, pl.ds(0, 2 * D)], 0)
    c_qkv = cp(wqkv_hbm, wqkv_v, 1)
    c_x = [cp(x_hbm.at[pl.ds(i * T1, T1)], x_v.at[pl.ds(i * T1, T1)], 8 + i)
           for i in range(S // T1)]
    c_wm1 = cp(wm_hbm.at[:, pl.ds(2 * D, 4 * D)], wm_v.at[:, pl.ds(2 * D, 4 * D)], 3)
    c_wo = cp(wo_hbm, wo_v, 4)
    c_wg = cp(wg_hbm, wg_v, 5)
    c_wu = cp(wu_hbm, wu_v, 6)
    c_wd = cp(wd_hbm, wd_v, 7)
    c_qkv.start(); c_wm0.start()
    for c_ in c_x:
        c_.start()

    cc = c_ref[...].astype(F32)
    sc = jnp.broadcast_to(cc * jax.nn.sigmoid(cc), (8, D)).astype(BF)

    r = jax.lax.broadcasted_iota(jnp.int32, (128, 128), 0)
    cidx = jax.lax.broadcasted_iota(jnp.int32, (128, 128), 1)
    same_head = (r // 16) == (cidx % 8)
    perm = jnp.where(same_head & ((r % 16) == (cidx // 8)), 1.0, 0.0).astype(BF)
    e = jnp.where(jax.lax.broadcasted_iota(jnp.int32, (16, 128), 0)
                  == jax.lax.broadcasted_iota(jnp.int32, (16, 128), 1) // 8, 1.0, 0.0).astype(BF)
    bds = [jnp.where(same_head, _dot(wphi_ref[g], e), 0.0).T.astype(BF) for g in range(G)]
    perm_t = perm.astype(F32).T.astype(BF)

    c_qkv.wait()
    c_wm1.start(); c_wo.start(); c_wg.start(); c_wu.start(); c_wd.start()
    for j in range(3):
        for g in range(G):
            o = j * D + g * 128
            m = perm_t if j == 2 else bds[g]
            wt_v[pl.ds(o, 128), :] = _dot(m, wqkv_v[:, pl.ds(o, 128)], NT).astype(BF)

    c_wm0.wait()
    mod_a = _dot(sc, wm_v[:, pl.ds(0, 2 * D)])[0:1]
    sa, ca = mod_a[:, :D], mod_a[:, D:]
    kv_v[...] = jnp.zeros(kv_v.shape, F32)

    def p1(i, _):
        c_x[i].wait()
        rows = pl.ds(i * T1, T1)
        h = _ln_mod(x_v[rows, :].astype(F32), ca, sa).astype(BF)
        h_v[rows, :] = h
        kvt = _dot(wt_v[pl.ds(D, 2 * D), :], h, NT)
        ones = jnp.ones((16, T1), BF)
        for g in range(G):
            pk = _phi(kvt[g * 128:(g + 1) * 128])
            v = kvt[D + g * 128:D + (g + 1) * 128].astype(BF)
            kv_v[g] += _dot(jnp.concatenate([v, ones], axis=0), pk, NT)
        return 0
    for i in range(S // T1):
        p1(i, 0)

    c_wo.wait()
    for g in range(G):
        wop_v[pl.ds(g * 128, 128), :] = _dot(perm_t, wo_v[pl.ds(g * 128, 128), :]).astype(BF)
    msk = (jax.lax.broadcasted_iota(jnp.int32, (144, 256), 0) % 8
           == jax.lax.broadcasted_iota(jnp.int32, (144, 256), 1) % 8)
    kvm = [jnp.where(msk, kv_v[g], 0.0).astype(BF) for g in range(G)]
    c_wm1.wait()
    mod_b = _dot(sc, wm_v[:, pl.ds(2 * D, 4 * D)])[0:1]
    ga, sb, cb, gb = (mod_b[:, j * D:(j + 1) * D] for j in range(4))
    c_wg.wait(); c_wu.wait(); c_wd.wait()

    def p2(i, _):
        rows = pl.ds(pl.multiple_of(i * T2, T2), T2)
        qt = _dot(wt_v[pl.ds(0, D), :], h_v[rows, :], NT)
        outs = []
        for g in range(G):
            nd = _dot(kvm[g], _phi(qt[g * 128:(g + 1) * 128]))
            inv = 1.0 / (nd[128:136] + 1e-6)
            outs.append((nd[:128].reshape(DH, 8, T2) * inv[None]).reshape(128, T2))
        ot = jnp.concatenate(outs, axis=0)
        o = ot.T.astype(BF)
        x1 = x_v[rows, :].astype(F32) + ga * _dot(o, wop_v[...])
        h2 = _ln_mod(x1, cb, sb).astype(BF)
        acc = None
        for f in range(F // FC):
            cs = pl.ds(f * FC, FC)
            a = jax.nn.gelu(_dot(h2, wg_v[:, cs]), approximate=True) * _dot(h2, wu_v[:, cs])
            d = _dot(a.astype(BF), wd_v[cs, :])
            acc = d if acc is None else acc + d
        out_v[rows, :] = (x1 + gb * acc).astype(out_v.dtype)
        pltpu.make_async_copy(out_v.at[rows, :], o_hbm.at[rows, :], osem.at[i]).start()
        return 0
    jax.lax.fori_loop(0, S // T2, p2, 0)
    for i in range(S // T2):
        rows = pl.ds(i * T2, T2)
        pltpu.make_async_copy(out_v.at[rows, :], o_hbm.at[rows, :], osem.at[i]).wait()


@jax.jit
def pallas_adaLN_cond__linear_kernel_hedgehog__geglu_ffn__prompt_kernel(
    A_x, A_wqkv, A_w_phi, A_wo, B_x, B_w_gate, B_w_up, B_w_down, c, w_mod,
):
    del B_x
    hbm = pl.BlockSpec(memory_space=pl.ANY)
    vm = pl.BlockSpec(memory_space=pltpu.VMEM)
    V = pltpu.VMEM
    out = pl.pallas_call(
        _kernel,
        in_specs=[hbm, hbm, vm, hbm, hbm, hbm, hbm, vm, hbm],
        out_specs=hbm,
        out_shape=jax.ShapeDtypeStruct((S, D), A_x.dtype),
        scratch_shapes=[
            V((S, D), BF), V((D, 3 * D), BF), V((D, D), BF), V((D, F), BF), V((D, F), BF),
            V((F, D), BF), V((D, 6 * D), BF), V((3 * D, D), BF), V((D, D), BF),
            V((S, D), BF), V((G, 144, 256), F32), V((S, D), A_x.dtype),
            pltpu.SemaphoreType.DMA((8 + S // T1,)), pltpu.SemaphoreType.DMA((S // T2,)),
        ],
        compiler_params=pltpu.CompilerParams(vmem_limit_bytes=100 * 1024 * 1024),
    )(A_x.reshape(S, D), A_wqkv, A_w_phi.reshape(G, 128, DH), A_wo,
      B_w_gate, B_w_up, B_w_down, c, w_mod)
    return out.reshape(A_x.shape)
```
